```python
import jax
import jax.numpy as jnp

def _softmax(x, axis=-1):
    return jax.nn.softmax(x, axis=axis)

def _gelu(x):
    return jax.nn.gelu(x, approximate=True)

def _silu(x):
    return jax.nn.silu(x)

def _sigmoid(x):
    return jax.nn.sigmoid(x)

def _layernorm(x, axis=-1, eps=1e-05):
    m = jnp.mean(x, axis=axis, keepdims=True)
    v = jnp.var(x, axis=axis, keepdims=True)
    return (x - m) / jnp.sqrt(v + eps)

def _scatter_add(tgt, idx, src, axis=0):
    return tgt.at[idx].add(src)

def _segment_sum(src, seg, n):
    return jax.ops.segment_sum(src, seg, n)

class _Rng:

    def __init__(self, key):
        self._k = key

    def _next(self):
        self._k, sub = jax.random.split(self._k)
        return sub

    def normal(self, shape):
        return jax.random.normal(self._next(), shape, dtype=jnp.bfloat16)

    def randint(self, lo, hi, shape):
        return jax.random.randint(self._next(), shape, lo, hi, dtype=jnp.int32)

    def uniform(self, shape, lo=0.0, hi=1.0):
        return jax.random.uniform(self._next(), shape, jnp.bfloat16, lo, hi)

    def permutation(self, n):
        return jax.random.permutation(self._next(), n)
kernel_name = 'recurrent_scan__memory_aug_recurrent_mem_tr__moe_arch_mod__prompt'

def setup_inputs():
    _rng = _Rng(jax.random.key(int.from_bytes(__import__("os").urandom(4), "little")))
    _w = lambda a: (lambda t: t.astype(jnp.bfloat16) if jnp.issubdtype(t.dtype, jnp.floating) else t)(jnp.asarray(a))

    def _A_setup():
        B, S, Dm = (1, 2048, 640)
        H, Dh = (32, 128)
        M, seg = (8, 32)
        seg = min(seg, S)
        S = S // seg * seg
        return {'x': _w((lambda *s: _rng.normal(s) * 0.05)(B, S, Dm)), 'mem0': _w((lambda *s: _rng.normal(s) * 0.05)(B, M, Dm)), 'Wq': _w((lambda *s: _rng.normal(s) * 0.05)(Dm, H, Dh) * Dm ** (-0.5)), 'Wk': _w((lambda *s: _rng.normal(s) * 0.05)(Dm, H, Dh) * Dm ** (-0.5)), 'Wv': _w((lambda *s: _rng.normal(s) * 0.05)(Dm, H, Dh) * Dm ** (-0.5)), 'Wo': _w((lambda *s: _rng.normal(s) * 0.05)(H, Dh, Dm) * (H * Dh) ** (-0.5)), 'seg_len': seg}
    _A_in = _A_setup()

    def _B_setup():
        B, S, D, F, C = (1, 2048, 640, 1728, 8)
        return {'x': _w((lambda *s: _rng.normal(s) * 0.05)(B, S, D)), 'w_r': _w((lambda *s: _rng.normal(s) * 0.05)(D)), 'w_gate': _w((lambda *s: _rng.normal(s) * 0.05)(D, F)), 'w_up': _w((lambda *s: _rng.normal(s) * 0.05)(D, F)), 'w_down': _w((lambda *s: _rng.normal(s) * 0.05)(F, D))}
    _B_in = _B_setup()
    return {'A_x': _A_in['x'], 'A_mem0': _A_in['mem0'], 'A_Wq': _A_in['Wq'], 'A_Wk': _A_in['Wk'], 'A_Wv': _A_in['Wv'], 'A_Wo': _A_in['Wo'], 'A_seg_len': _A_in['seg_len'], 'B_x': _B_in['x'], 'B_w_r': _B_in['w_r'], 'B_w_gate': _B_in['w_gate'], 'B_w_up': _B_in['w_up'], 'B_w_down': _B_in['w_down']}

def reference(A_x, A_mem0, A_Wq, A_Wk, A_Wv, A_Wo, A_seg_len, B_x, B_w_r, B_w_gate, B_w_up, B_w_down):

    def _A_ref(x, mem0, Wq, Wk, Wv, Wo, seg_len):
        B, S, Dm = x.shape
        H, Dh = (Wq.shape[1], Wq.shape[2])
        M = mem0.shape[1]
        scale = Dh ** (-0.5)
        n_seg = S // seg_len
        L = M + seg_len
        idx = jnp.arange(L)
        mask = (idx[:, None] < M) | (idx[:, None] >= idx[None, :])
        mem = mem0
        outs = []
        for s in range(n_seg):
            xs = x[:, s * seg_len:(s + 1) * seg_len, :].copy()
            h = jnp.concatenate([mem, xs], axis=1)
            q = jnp.einsum('btd,dhe->bhte', h, Wq)
            k = jnp.einsum('btd,dhe->bhte', h, Wk)
            v = jnp.einsum('btd,dhe->bhte', h, Wv)
            scores = jnp.einsum('bhqe,bhke->bhqk', q, k) * scale
            scores = jnp.where(mask[None, None], scores, -1000000000.0)
            p = _softmax(scores, axis=-1)
            o = jnp.einsum('bhqk,bhke->bhqe', p, v)
            o = jnp.einsum('bhte,hed->btd', o, Wo)
            mem = o[:, :M, :].copy()
            outs.append(o[:, M:, :])
        return jnp.concatenate(outs, axis=1)

    def _B_ref(x, w_r, w_gate, w_up, w_down):
        B, S, D = x.shape
        C = 8
        r = x @ w_r
        idx = jnp.argsort(-r, axis=-1)[:, :C]
        idx_e = jnp.repeat(idx.reshape(B, C, 1), D, axis=2)
        x_sel = jnp.take_along_axis(x, idx_e, axis=1)
        g = _silu(x_sel @ w_gate)
        u = x_sel @ w_up
        y = g * u @ w_down
        r_sel = _sigmoid(jnp.take_along_axis(r, idx, axis=1))
        y = y * r_sel.reshape(B, C, 1)
        b_off = (jnp.arange(B) * S).reshape(B, 1)
        flat_idx = (idx + b_off).reshape(B * C)
        zero = (x * 0.0).reshape(B * S, D)
        upd = _scatter_add(zero, flat_idx, y.reshape(B * C, D), axis=0)
        return x + upd.reshape(B, S, D)
    x = A_x
    xn = _layernorm(x, axis=-1)
    s = _A_ref(xn, A_mem0, A_Wq, A_Wk, A_Wv, A_Wo, A_seg_len)
    g = _silu(_B_ref(xn, B_w_r, B_w_gate, B_w_up, B_w_down))
    return x + s * g
```

```python
import functools

import jax
import jax.numpy as jnp
import numpy as np
from jax import lax
from jax.experimental import pallas as pl
from jax.experimental.pallas import tpu as pltpu

F32 = jnp.float32
BF16 = jnp.bfloat16
U32 = jnp.uint32

TOP_C = 8
HOIST = 8
HEAD_CHUNK = 16
GROUP = 4
LAG_QK = 1
LAG_PV = 1
O_GROUP = 8
DENSE_M = 256
DENSE_HEADS = 4
LN_ROWS = 256


def _dot(a, b):
    return lax.dot_general(a, b, (((1,), (0,)), ((), ())), preferred_element_type=F32)


def _dot_nt(a, b):
    return lax.dot_general(a, b, (((1,), (1,)), ((), ())), preferred_element_type=F32)


def _round(x):
    return x.astype(BF16).astype(F32)


def _silu(x):
    return x * jax.nn.sigmoid(x)


def _layernorm(x):
    n = x.shape[-1]
    mean = jnp.sum(x, axis=-1, keepdims=True) / n
    cen = x - mean
    var = jnp.sum(cen * cen, axis=-1, keepdims=True) / n
    eps = float(np.asarray(1e-5, dtype=BF16))
    sd = _round(jnp.sqrt(_round(_round(var) + eps)))
    return (_round(x - _round(mean)) / sd).astype(BF16)


def _pack_heads(w):
    u = pltpu.bitcast(w, U32)
    u = u.reshape(8, 2, 8, 128)
    a, b = u[:, 0], u[:, 1]
    even = (a & jnp.uint32(0xFFFF)) | (b << 16)
    odd = (a >> 16) | (b & jnp.uint32(0xFFFF0000))
    even = jnp.swapaxes(even, 0, 1)
    odd = jnp.swapaxes(odd, 0, 1)
    return [(odd if h % 2 else even)[h // 2] for h in range(16)]


def _kernel(x_hbm, mem0_hbm, wq_hbm, wk_hbm, wv_hbm, wo_hbm, wr_hbm, wg_hbm, wu_hbm, wd_hbm,
            out_hbm,
            x_v, mem0_v, wr_v, xn_v, gate_v, xh_v, stage, wqkv, wo_stage, wo_v, hz, wg_v, wu_v, wd_v,
            out_v, xsel_v, w_sems, misc_sems, out_sem, *, seg):
    S, D = x_v.shape
    M = mem0_v.shape[0]
    H, DH = wq_hbm.shape[1], wq_hbm.shape[2]
    n_seg = S // seg
    L = M + seg
    live = seg - HOIST
    n_chunk = H // HEAD_CHUNK

    x_cp = pltpu.make_async_copy(x_hbm, x_v, misc_sems.at[0])
    x_cp.start()
    for m, w_hbm in enumerate((wq_hbm, wk_hbm, wv_hbm)):
        for c in range(n_chunk):
            i = m * n_chunk + c
            pltpu.make_async_copy(w_hbm.at[:, pl.ds(c * HEAD_CHUNK, HEAD_CHUNK), :],
                                  stage.at[i], w_sems.at[i]).start()
    wo_cp = pltpu.make_async_copy(wo_hbm, wo_stage, misc_sems.at[1])
    wg_cp = pltpu.make_async_copy(wg_hbm, wg_v, misc_sems.at[2])
    wu_cp = pltpu.make_async_copy(wu_hbm, wu_v, misc_sems.at[3])
    wd_cp = pltpu.make_async_copy(wd_hbm, wd_v, misc_sems.at[4])
    mem0_cp = pltpu.make_async_copy(mem0_hbm, mem0_v, misc_sems.at[5])
    wr_cp = pltpu.make_async_copy(wr_hbm, wr_v, misc_sems.at[6])
    for cp in (wo_cp, mem0_cp, wr_cp, wg_cp, wu_cp, wd_cp):
        cp.start()

    x_cp.wait()

    def ln_body(i, _):
        r0 = pl.multiple_of(i * LN_ROWS, LN_ROWS)
        xn = _layernorm(x_v[pl.ds(r0, LN_ROWS), :].astype(F32)).astype(F32)
        xn_v[pl.ds(r0, LN_ROWS), :] = xn
        gate_v[pl.ds(r0, LN_ROWS), :] = _silu(xn)
        per = LN_ROWS // seg
        hoisted = jnp.concatenate(
            [xn[j * seg + live:(j + 1) * seg] for j in range(per)], axis=0)
        h0 = pl.multiple_of(i * (per * HOIST), per * HOIST)
        xh_v[pl.ds(h0, per * HOIST), :] = hoisted.astype(BF16)

    lax.fori_loop(0, S // LN_ROWS, ln_body, None)

    def chunk_body(i, _):
        m = i // n_chunk
        h0 = (i % n_chunk) * HEAD_CHUNK
        pltpu.make_async_copy(wq_hbm.at[:, pl.ds(0, HEAD_CHUNK), :], stage.at[i],
                              w_sems.at[i]).wait()

        def repack(j, _):
            d0 = pl.multiple_of(j * 16, 16)
            r0 = pl.multiple_of(j * 8, 8)
            for h, w in enumerate(_pack_heads(stage[i, pl.ds(d0, 16)])):
                wqkv[(h0 + h) * 3 + m, pl.ds(r0, 8), :] = w

        lax.fori_loop(0, D // 16, repack, None)

        def project(j, _):
            hb = h0 + j * DENSE_HEADS
            w = jnp.concatenate(
                [pltpu.bitcast(wqkv[(hb + h) * 3 + m], BF16) for h in range(DENSE_HEADS)],
                axis=1)
            for r in range(0, n_seg * HOIST, DENSE_M):
                y = _dot(xh_v[r:r + DENSE_M, :], w)
                for h in range(DENSE_HEADS):
                    hz[(hb + h) * 3 + m, r:r + DENSE_M, :] = y[:, h * DH:(h + 1) * DH]

        lax.fori_loop(0, HEAD_CHUNK // DENSE_HEADS, project, None)

    lax.fori_loop(0, 3 * n_chunk, chunk_body, None)

    wo_cp.wait()

    def wo_body(i, _):
        r0 = pl.multiple_of(i * 256, 256)
        p0 = pl.multiple_of(i * 128, 128)
        wo_v[pl.ds(p0, 128), :] = pltpu.bitcast(wo_stage[pl.ds(r0, 256), :], U32)

    lax.fori_loop(0, H * DH // 256, wo_body, None)

    wr_cp.wait()
    w_r = wr_v[...].astype(F32)
    w_r = jnp.concatenate(
        [jnp.broadcast_to(w_r[k:k + 1], (8, 128)) for k in range(D // 128)], axis=1)
    score = _round(_dot_nt(w_r, xn_v[...].astype(BF16)))
    pos = lax.broadcasted_iota(jnp.int32, (8, S), 1).astype(F32)
    slot = lax.broadcasted_iota(jnp.int32, (TOP_C, 1), 0)
    free = jnp.ones((8, S), jnp.int32)
    r_sel = jnp.zeros((TOP_C, 1), F32)
    picked = []
    for c in range(TOP_C):
        cand = jnp.where(free > 0, score, -jnp.inf)
        best = jnp.max(cand, axis=1, keepdims=True)
        first = jnp.min(jnp.where((cand == best) & (free > 0), pos, float(S)),
                        axis=1, keepdims=True)
        free = jnp.where(pos == first, 0, free)
        r_sel = jnp.where(slot == c, best, r_sel)
        idx = jnp.clip(jnp.max(first).astype(jnp.int32), 0, S - 1)
        picked.append(idx)
        xsel_v[c:c + 1, :] = xn_v[pl.ds(idx, 1), :]

    wg_cp.wait()
    wu_cp.wait()
    wd_cp.wait()
    x_sel = xsel_v[...]
    act = _round(_silu(_round(_dot_nt(x_sel, wg_v[...]))))
    up = _round(_dot_nt(x_sel, wu_v[...]))
    y = _round(_dot(_round(act * up), wd_v[...]))
    y = _round(y * _round(jax.nn.sigmoid(r_sel)))
    g_sel = _silu(_round(x_sel + y))
    for c in range(TOP_C):
        gate_v[pl.ds(picked[c], 1), :] = g_sel[c:c + 1, :]

    n_grp = H // GROUP
    key_pad = -L % 16
    exp_scale = float(DH ** -0.5 * np.log2(np.e))

    def step(s, mem):
        base = pl.multiple_of(s * seg, seg)
        zb = pl.multiple_of(s * HOIST, HOIST)
        h_in = jnp.concatenate([mem, xn_v[pl.ds(base, live), :]], axis=0).astype(BF16)

        row = lax.broadcasted_iota(jnp.int32, (L, L + key_pad), 0)
        col = lax.broadcasted_iota(jnp.int32, (L, L + key_pad), 1)
        visible = ((row < M) | (row >= col)) & (col < L)
        fill = jnp.where(col < L, -1e9 * DH ** 0.5, -jnp.inf).astype(F32)

        qkv, prob, ctx, acc = {}, {}, {}, []

        def keys(t):
            return jnp.concatenate([t, jnp.zeros((key_pad, DH), F32)], axis=0).astype(BF16)

        def project(g):
            lo = g * GROUP * 3
            w = jnp.concatenate(
                [pltpu.bitcast(wqkv[lo + j], BF16) for j in range(GROUP * 3)], axis=1)
            y = _dot(h_in, w)
            for j in range(GROUP * 3):
                qkv[lo + j] = jnp.concatenate(
                    [y[:, j * DH:(j + 1) * DH], hz[lo + j, pl.ds(zb, HOIST), :]], axis=0)

        def scores(g):
            for h in range(g * GROUP, (g + 1) * GROUP):
                sc = _dot_nt(_round(qkv[3 * h]), keys(qkv[3 * h + 1]))
                sc = jnp.where(visible, sc, fill)
                e = jnp.exp2((sc - jnp.max(sc, axis=1, keepdims=True)) * exp_scale)
                prob[h] = _round(e / jnp.sum(e, axis=1, keepdims=True))

        def values(g):
            for h in range(g * GROUP, (g + 1) * GROUP):
                ctx[h] = _round(_dot(prob[h], keys(qkv[3 * h + 2])))

        def out_proj(og):
            o = jnp.concatenate(
                [ctx[h] for h in range(og * O_GROUP, (og + 1) * O_GROUP)], axis=1)
            rows = O_GROUP * DH // 2
            acc.append(_dot(o, pltpu.bitcast(wo_v[og * rows:(og + 1) * rows, :], BF16)))

        for t in range(n_grp + LAG_QK + LAG_PV):
            if t < n_grp:
                project(t)
            if 0 <= t - LAG_QK < n_grp:
                scores(t - LAG_QK)
            if t >= n_grp:
                while (len(acc) + 1) * O_GROUP <= (t - LAG_QK - LAG_PV) * GROUP:
                    out_proj(len(acc))
            if 0 <= t - LAG_QK - LAG_PV < n_grp:
                values(t - LAG_QK - LAG_PV)
        while len(acc) * O_GROUP < H:
            out_proj(len(acc))

        o = functools.reduce(lambda a, b: a + b, acc)
        x_seg = x_v[pl.ds(base, seg), :].astype(F32)
        out_v[pl.ds(base, seg), :] = (
            x_seg + o[M:] * gate_v[pl.ds(base, seg), :]).astype(BF16)
        pltpu.make_async_copy(out_v.at[pl.ds(base, seg), :],
                              out_hbm.at[pl.ds(base, seg), :], out_sem).start()
        return _round(o[:M])

    mem0_cp.wait()
    lax.fori_loop(0, n_seg, step, mem0_v[...].astype(F32))
    pltpu.make_async_copy(out_v, out_hbm, out_sem).wait()


@functools.partial(jax.jit, static_argnames=("A_seg_len",))
def pallas_recurrent_scan__memory_aug_recurrent_mem_tr__moe_arch_mod__prompt_kernel(
    A_x: jax.Array,
    A_mem0: jax.Array,
    A_Wq: jax.Array,
    A_Wk: jax.Array,
    A_Wv: jax.Array,
    A_Wo: jax.Array,
    A_seg_len: int,
    B_x: jax.Array,
    B_w_r: jax.Array,
    B_w_gate: jax.Array,
    B_w_up: jax.Array,
    B_w_down: jax.Array,
):
    del B_x
    B, S, D = A_x.shape
    M = A_mem0.shape[1]
    _, H, DH = A_Wq.shape
    F = B_w_gate.shape[1]
    seg = int(A_seg_len)
    assert B == 1 and M == 8 and DH == 128 and seg % 16 == 0 and S % LN_ROWS == 0
    n_hoist = S // seg * HOIST

    hbm = pl.BlockSpec(memory_space=pltpu.HBM)
    out = pl.pallas_call(
        functools.partial(_kernel, seg=seg),
        out_shape=jax.ShapeDtypeStruct((S, D), A_x.dtype),
        in_specs=[hbm] * 10,
        out_specs=hbm,
        scratch_shapes=[
            pltpu.VMEM((S, D), BF16),
            pltpu.VMEM((M, D), BF16),
            pltpu.VMEM((D // 128, 128), BF16),
            pltpu.VMEM((S, D), F32),
            pltpu.VMEM((S, D), F32),
            pltpu.VMEM((n_hoist, D), BF16),
            pltpu.VMEM((3 * H // HEAD_CHUNK, D, HEAD_CHUNK, DH), BF16),
            pltpu.VMEM((3 * H, D // 2, DH), U32),
            pltpu.VMEM((H * DH, D), BF16),
            pltpu.VMEM((H * DH // 2, D), U32),
            pltpu.VMEM((3 * H, n_hoist, DH), F32),
            pltpu.VMEM((F, D), BF16),
            pltpu.VMEM((F, D), BF16),
            pltpu.VMEM((F, D), BF16),
            pltpu.VMEM((S, D), BF16),
            pltpu.VMEM((TOP_C, D), F32),
            pltpu.SemaphoreType.DMA((3 * H // HEAD_CHUNK,)),
            pltpu.SemaphoreType.DMA((7,)),
            pltpu.SemaphoreType.DMA(()),
        ],
        compiler_params=pltpu.CompilerParams(vmem_limit_bytes=112 * 1024 * 1024),
    )(A_x.reshape(S, D), A_mem0.reshape(M, D), A_Wq, A_Wk, A_Wv, A_Wo.reshape(H * DH, D),
      B_w_r.reshape(D // 128, 128), B_w_gate.T, B_w_up.T, B_w_down)
    return out.reshape(B, S, D)
```

```python
import functools

import jax
import jax.numpy as jnp
import numpy as np
from jax import lax
from jax.experimental import pallas as pl
from jax.experimental.pallas import tpu as pltpu

F32 = jnp.float32
BF16 = jnp.bfloat16
U32 = jnp.uint32

TOP_C = 8
HOIST = 8
AHEAD = 2
FFN_PIECES = 12
GROUP = 4
LAG_QK = 1
LAG_PV = 1
O_GROUP = 8
PROFILE = 0


def _scope(name):
    import contextlib
    return jax.named_scope(name) if PROFILE else contextlib.nullcontext()


def _dot(a, b):
    return lax.dot_general(a, b, (((1,), (0,)), ((), ())), preferred_element_type=F32)


def _dot_nt(a, b):
    return lax.dot_general(a, b, (((1,), (1,)), ((), ())), preferred_element_type=F32)


def _round(x):
    return x.astype(BF16).astype(F32)


def _silu(x):
    h = 0.5 * x
    return h + h * jnp.tanh(h)


def _layernorm(x):
    n = x.shape[-1]
    mean = jnp.sum(x, axis=-1, keepdims=True) / n
    cen = x - mean
    var = jnp.sum(cen * cen, axis=-1, keepdims=True) / n
    eps = float(np.asarray(1e-5, dtype=BF16))
    sd = _round(jnp.sqrt(_round(_round(var) + eps)))
    return _round(_round(x - _round(mean)) * (1.0 / sd))


def _kernel(x_hbm, mem0_hbm, wq_hbm, wk_hbm, wv_hbm, wo_hbm, wr_hbm, wg_hbm, wu_hbm, wd_hbm,
            out_hbm,
            x_v, xh_raw, mem0_v, wr_v, xn_v, gin_v, xh_v, stage, wqkv, wo_stage, wo_v, hz,
            wg_v, wu_v, wd_v, out_v, xsel_v, x_sems, w_sems, misc_sems, out_sem):
    n_seg, seg, D = x_v.shape
    S = n_seg * seg
    M = mem0_v.shape[0]
    H, DH = wq_hbm.shape[1], wq_hbm.shape[2]
    L = M + seg
    live = seg - HOIST
    n_iter = H // 2
    segs = n_seg // n_iter

    words = [w.bitcast(U32) for w in (wq_hbm, wk_hbm, wv_hbm)]
    wo_rows = H * DH // n_iter
    ffn_rows = wg_v.shape[0] // FFN_PIECES

    def late_copies(i):
        wo_at = pl.ds(pl.multiple_of(i * wo_rows, wo_rows), wo_rows)
        return [pltpu.make_async_copy(wo_hbm.at[wo_at], wo_stage.at[wo_at], misc_sems.at[1])]

    def ffn_copies(i):
        at = pl.ds(pl.multiple_of(i * ffn_rows, ffn_rows), ffn_rows)
        return [pltpu.make_async_copy(src.at[at], dst.at[at], misc_sems.at[2 + k])
                for k, (src, dst) in enumerate(((wg_hbm, wg_v), (wu_hbm, wu_v), (wd_hbm, wd_v)))]

    def start_iteration(i):
        for m in range(3):
            pltpu.make_async_copy(words[m].at[:, i, :], stage.at[i, m], w_sems.at[i]).start()
        at = pl.ds(i * segs, segs)
        pltpu.make_async_copy(x_hbm.at[at], x_v.at[at], x_sems.at[i]).start()

    xh_cp = pltpu.make_async_copy(x_hbm.at[:, pl.ds(live, HOIST), :], xh_raw, misc_sems.at[0])
    mem0_cp = pltpu.make_async_copy(mem0_hbm, mem0_v, misc_sems.at[5])
    wr_cp = pltpu.make_async_copy(wr_hbm, wr_v, misc_sems.at[6])
    xh_cp.start()
    start_iteration(0)

    with _scope("xh_wait"):
        xh_cp.wait()
    for i in range(1, AHEAD):
        start_iteration(i)
    mem0_cp.start()
    wr_cp.start()

    def xh_body(i, _):
        s0 = pl.multiple_of(i * 16, 16)
        rows = xh_raw[pl.ds(s0, 16)].astype(F32).reshape(16 * HOIST, D)
        r0 = pl.multiple_of(i * (16 * HOIST), 16 * HOIST)
        xh_v[pl.ds(r0, 16 * HOIST), :] = _layernorm(rows).astype(BF16)

    with _scope("xh_ln"):
        lax.fori_loop(0, n_seg // 16, xh_body, None)

    def dense_body(i, _):
        pltpu.make_async_copy(stage.at[i], stage.at[i], w_sems.at[i]).wait()
        s0 = i * segs
        got = x_v.at[pl.ds(s0, segs)]
        pltpu.make_async_copy(got, got, x_sems.at[i]).wait()

        @pl.when(i + AHEAD < n_iter)
        def _():
            start_iteration(i + AHEAD)

        for cp in late_copies(i):
            cp.start()

        @pl.when(i < FFN_PIECES)
        def _():
            for cp in ffn_copies(i):
                cp.start()

        for m in range(3):
            a = stage[i, m, pl.ds(0, D // 2, stride=2), :]
            b = stage[i, m, pl.ds(1, D // 2, stride=2), :]
            even = (a & jnp.uint32(0xFFFF)) | (b << 16)
            odd = (a >> 16) | (b & jnp.uint32(0xFFFF0000))
            head = m * H + 2 * i
            wqkv[head] = even
            wqkv[head + 1] = odd
            w = jnp.concatenate(
                [pltpu.bitcast(even, BF16), pltpu.bitcast(odd, BF16)], axis=1)
            y = _dot(xh_v[...], w)
            hz[head] = y[:, :DH]
            hz[head + 1] = y[:, DH:]

        xn = _layernorm(x_v[pl.ds(s0, segs)].astype(F32).reshape(segs * seg, D))
        r0 = pl.multiple_of(s0 * seg, segs * seg)
        xn_v[pl.ds(r0, segs * seg), :] = xn
        gin_v[pl.ds(r0, segs * seg), :] = xn

    with _scope("dense"):
        lax.fori_loop(0, n_iter, dense_body, None)

    pltpu.make_async_copy(wo_hbm, wo_stage, misc_sems.at[1]).wait()

    def wo_body(i, _):
        r0 = pl.multiple_of(i * 256, 256)
        p0 = pl.multiple_of(i * 128, 128)
        wo_v[pl.ds(p0, 128), :] = pltpu.bitcast(wo_stage[pl.ds(r0, 256), :], U32)

    with _scope("wo"):
        lax.fori_loop(0, H * DH // 256, wo_body, None)

    wr_cp.wait()
    w_r = wr_v[...].astype(F32)
    w_r = jnp.concatenate(
        [jnp.broadcast_to(w_r[k:k + 1], (8, 128)) for k in range(D // 128)], axis=1)
    score = _round(_dot_nt(w_r, xn_v[...].astype(BF16)))
    pos = lax.broadcasted_iota(jnp.int32, (8, S), 1).astype(F32)
    slot = lax.broadcasted_iota(jnp.int32, (TOP_C, 1), 0)
    free = jnp.ones((8, S), jnp.int32)
    r_sel = jnp.zeros((TOP_C, 1), F32)
    picked = []
    for c in range(TOP_C):
        cand = jnp.where(free > 0, score, -jnp.inf)
        best = jnp.max(cand, axis=1, keepdims=True)
        first = jnp.min(jnp.where((cand == best) & (free > 0), pos, float(S)),
                        axis=1, keepdims=True)
        free = jnp.where(pos == first, 0, free)
        r_sel = jnp.where(slot == c, best, r_sel)
        idx = jnp.clip(jnp.max(first).astype(jnp.int32), 0, S - 1)
        picked.append(idx)
        xsel_v[c:c + 1, :] = xn_v[pl.ds(idx, 1), :]

    pltpu.make_async_copy(wg_hbm, wg_v, misc_sems.at[2]).wait()
    pltpu.make_async_copy(wu_hbm, wu_v, misc_sems.at[3]).wait()
    pltpu.make_async_copy(wd_hbm, wd_v, misc_sems.at[4]).wait()
    x_sel = xsel_v[...]
    act = _round(_silu(_round(_dot_nt(x_sel, wg_v[...]))))
    up = _round(_dot_nt(x_sel, wu_v[...]))
    y = _round(_dot(_round(act * up), wd_v[...]))
    y = _round(y * _round(jax.nn.sigmoid(r_sel)))
    g_in = _round(x_sel + y)
    for c in range(TOP_C):
        gin_v[pl.ds(picked[c], 1), :] = g_in[c:c + 1, :]

    n_grp = H // GROUP
    key_pad = -L % 16
    exp_scale = float(DH ** -0.5 * np.log2(np.e))

    def step(s, mem):
        base = pl.multiple_of(s * seg, seg)
        zb = pl.multiple_of(s * HOIST, HOIST)
        h_in = jnp.concatenate([mem, xn_v[pl.ds(base, live), :]], axis=0).astype(BF16)

        row = lax.broadcasted_iota(jnp.int32, (L, L + key_pad), 0)
        col = lax.broadcasted_iota(jnp.int32, (L, L + key_pad), 1)
        visible = ((row < M) | (row >= col)) & (col < L)
        fill = jnp.where(col < L, -1e9 * DH ** 0.5, -jnp.inf).astype(F32)

        qkv, prob, ctx, acc = {}, {}, {}, []

        def keys(t):
            return jnp.concatenate([t, jnp.zeros((key_pad, DH), F32)], axis=0).astype(BF16)

        def project(g):
            ids = [m * H + h for h in range(g * GROUP, (g + 1) * GROUP) for m in range(3)]
            y = _dot(h_in, jnp.concatenate(
                [pltpu.bitcast(wqkv[i], BF16) for i in ids], axis=1))
            for j, i in enumerate(ids):
                qkv[i] = jnp.concatenate(
                    [y[:, j * DH:(j + 1) * DH], hz[i, pl.ds(zb, HOIST), :]], axis=0)

        def scores(g):
            for h in range(g * GROUP, (g + 1) * GROUP):
                sc = _dot_nt(_round(qkv[h]), keys(qkv[H + h]))
                sc = jnp.where(visible, sc, fill)
                e = jnp.exp2((sc - jnp.max(sc, axis=1, keepdims=True)) * exp_scale)
                prob[h] = _round(e / jnp.sum(e, axis=1, keepdims=True))

        def values(g):
            for h in range(g * GROUP, (g + 1) * GROUP):
                ctx[h] = _round(_dot(prob[h], keys(qkv[2 * H + h])))

        def out_proj(og):
            o = jnp.concatenate(
                [ctx[h] for h in range(og * O_GROUP, (og + 1) * O_GROUP)], axis=1)
            rows = O_GROUP * DH // 2
            acc.append(_dot(o, pltpu.bitcast(wo_v[og * rows:(og + 1) * rows, :], BF16)))

        for t in range(n_grp + LAG_QK + LAG_PV):
            if t < n_grp:
                project(t)
            if 0 <= t - LAG_QK < n_grp:
                scores(t - LAG_QK)
            if t >= n_grp:
                while (len(acc) + 1) * O_GROUP <= (t - LAG_QK - LAG_PV) * GROUP:
                    out_proj(len(acc))
            if 0 <= t - LAG_QK - LAG_PV < n_grp:
                values(t - LAG_QK - LAG_PV)
        while len(acc) * O_GROUP < H:
            out_proj(len(acc))

        o = functools.reduce(lambda a, b: a + b, acc)
        gate = _silu(gin_v[pl.ds(base, seg), :])
        out_v[s] = (x_v[s].astype(F32) + o[M:] * gate).astype(BF16)
        pltpu.make_async_copy(out_v.at[s], out_hbm.at[s], out_sem).start()
        return _round(o[:M])

    mem0_cp.wait()
    with _scope("steps"):
        lax.fori_loop(0, n_seg, step, mem0_v[...].astype(F32))
    pltpu.make_async_copy(out_v, out_hbm, out_sem).wait()


@functools.partial(jax.jit, static_argnames=("A_seg_len",))
def pallas_recurrent_scan__memory_aug_recurrent_mem_tr__moe_arch_mod__prompt_kernel(
    A_x: jax.Array,
    A_mem0: jax.Array,
    A_Wq: jax.Array,
    A_Wk: jax.Array,
    A_Wv: jax.Array,
    A_Wo: jax.Array,
    A_seg_len: int,
    B_x: jax.Array,
    B_w_r: jax.Array,
    B_w_gate: jax.Array,
    B_w_up: jax.Array,
    B_w_down: jax.Array,
):
    del B_x
    B, S, D = A_x.shape
    M = A_mem0.shape[1]
    _, H, DH = A_Wq.shape
    F = B_w_gate.shape[1]
    seg = int(A_seg_len)
    n_seg = S // seg
    assert B == 1 and M == 8 and DH == 128 and seg % 16 == 0 and n_seg * seg == S

    hbm = pl.BlockSpec(memory_space=pltpu.HBM)
    out = pl.pallas_call(
        _kernel,
        out_shape=jax.ShapeDtypeStruct((n_seg, seg, D), A_x.dtype),
        in_specs=[hbm] * 10,
        out_specs=hbm,
        scratch_shapes=[
            pltpu.VMEM((n_seg, seg, D), BF16),
            pltpu.VMEM((n_seg, HOIST, D), BF16),
            pltpu.VMEM((M, D), BF16),
            pltpu.VMEM((D // 128, 128), BF16),
            pltpu.VMEM((S, D), F32),
            pltpu.VMEM((S, D), F32),
            pltpu.VMEM((n_seg * HOIST, D), BF16),
            pltpu.VMEM((H // 2, 3, D, DH), U32),
            pltpu.VMEM((3 * H, D // 2, DH), U32),
            pltpu.VMEM((H * DH, D), BF16),
            pltpu.VMEM((H * DH // 2, D), U32),
            pltpu.VMEM((3 * H, n_seg * HOIST, DH), F32),
            pltpu.VMEM((F, D), BF16),
            pltpu.VMEM((F, D), BF16),
            pltpu.VMEM((F, D), BF16),
            pltpu.VMEM((n_seg, seg, D), BF16),
            pltpu.VMEM((TOP_C, D), F32),
            pltpu.SemaphoreType.DMA((H // 2,)),
            pltpu.SemaphoreType.DMA((H // 2,)),
            pltpu.SemaphoreType.DMA((7,)),
            pltpu.SemaphoreType.DMA(()),
        ],
        compiler_params=pltpu.CompilerParams(vmem_limit_bytes=112 * 1024 * 1024),
    )(A_x.reshape(n_seg, seg, D), A_mem0.reshape(M, D), A_Wq, A_Wk, A_Wv,
      A_Wo.reshape(H * DH, D), B_w_r.reshape(D // 128, 128), B_w_gate.T, B_w_up.T, B_w_down)
    return out.reshape(B, S, D)
```

```python
import functools

import jax
import jax.numpy as jnp
import numpy as np
from jax import lax
from jax.experimental import pallas as pl
from jax.experimental.pallas import tpu as pltpu

F32 = jnp.float32
BF16 = jnp.bfloat16
U32 = jnp.uint32

TOP_C = 8
HOIST = 8
FFN_PIECES = 6
AHEAD = 3
GROUP = 4
LAG_QK = 1
LAG_PV = 1
TAIL = "S7-O0:2-O2:4-V6-V7-O4:6-O6:8"
UNROLL = 8
ORDER_A = "n012rs"
ORDER_B = "0p1w2s"
K_MAJOR = 1
N_MAJOR = 1
PROFILE = 0


def _scope(name):
    import contextlib
    return jax.named_scope(name) if PROFILE else contextlib.nullcontext()


def _dot(a, b):
    return lax.dot_general(a, b, (((1,), (0,)), ((), ())), preferred_element_type=F32)


def _dot_nt(a, b):
    return lax.dot_general(a, b, (((1,), (1,)), ((), ())), preferred_element_type=F32)


def _round(x):
    return x.astype(BF16).astype(F32)


def _silu(x):
    h = 0.5 * x
    return h + h * jnp.tanh(h)


def _layernorm(x):
    inv_n = 1.0 / x.shape[-1]
    mean = jnp.sum(x, axis=-1, keepdims=True) * inv_n
    cen = x - mean
    var = jnp.sum(cen * cen, axis=-1, keepdims=True) * inv_n
    eps = float(np.asarray(1e-5, dtype=BF16))
    sd = _round(jnp.sqrt(_round(_round(var) + eps)))
    return _round(_round(x - _round(mean)) * (1.0 / sd))


def _kernel(x_hbm, mem0_hbm, wq_hbm, wk_hbm, wv_hbm, wo_hbm, wr_hbm, wg_hbm, wu_hbm, wd_hbm,
            out_hbm,
            x_v, xh_raw, mem0_v, wr_v, xn_v, gin_v, xh_v, stage, wqkv, wo_stage, wo_v, hz,
            wg_v, wu_v, wd_v, out_v, score_v, xsel_v, rsel_v, picked_s,
            x_sems, w_sems, wo_sems, misc_sems, out_sem):
    n_seg, seg, D = x_v.shape
    S = n_seg * seg
    M = mem0_v.shape[0]
    H, DH = wq_hbm.shape[1], wq_hbm.shape[2]
    L = M + seg
    live = seg - HOIST
    n_pair = H // 2
    n_norm = n_pair - TOP_C
    segs = n_seg // n_norm
    block = segs * seg

    words = [w.bitcast(U32) for w in (wq_hbm, wk_hbm, wv_hbm)]

    def start_pair(i):
        for m in range(3):
            pltpu.make_async_copy(words[m].at[:, i, :], stage.at[i, m], w_sems.at[i]).start()

    def start_x(i):
        at = pl.ds(i * segs, segs)
        pltpu.make_async_copy(x_hbm.at[at], x_v.at[at], x_sems.at[i]).start()

    def piece(src, dst, sem, i, n):
        rows = dst.shape[0] // n
        at = pl.ds(pl.multiple_of(i * rows, 8), rows)
        return pltpu.make_async_copy(src.at[at], dst.at[at], sem)

    xh_cp = pltpu.make_async_copy(x_hbm.at[:, pl.ds(live, HOIST), :], xh_raw, misc_sems.at[0])
    mem0_cp = pltpu.make_async_copy(mem0_hbm, mem0_v, misc_sems.at[5])
    wr_cp = pltpu.make_async_copy(wr_hbm, wr_v, misc_sems.at[6])
    xh_cp.start()
    start_pair(0)
    start_x(0)
    wr_cp.start()

    with _scope("xh_wait"):
        xh_cp.wait()
    for i in range(1, AHEAD):
        start_pair(i)
        start_x(i)
    mem0_cp.start()

    def xh_body(i, _):
        s0 = pl.multiple_of(i * 16, 16)
        rows = xh_raw[pl.ds(s0, 16)].astype(F32).reshape(16 * HOIST, D)
        r0 = pl.multiple_of(i * (16 * HOIST), 16 * HOIST)
        xh_v[pl.ds(r0, 16 * HOIST), :] = _layernorm(rows).astype(BF16)

    with _scope("xh_ln"):
        lax.fori_loop(0, n_seg // 16, xh_body, None)
    wr_cp.wait()

    def project_pair(i, m):
        a = stage[i, m, pl.ds(0, D // 2, stride=2), :]
        b = stage[i, m, pl.ds(1, D // 2, stride=2), :]
        even = (a & jnp.uint32(0xFFFF)) | (b << 16)
        odd = (a >> 16) | (b & jnp.uint32(0xFFFF0000))
        head = m * H + 2 * i
        wqkv[head] = even
        wqkv[head + 1] = odd
        w = jnp.concatenate([pltpu.bitcast(even, BF16), pltpu.bitcast(odd, BF16)], axis=1)
        y = _dot(xh_v[...], w)
        hz[head] = y[:, :DH]
        hz[head + 1] = y[:, DH:]

    def wait_pair(i):
        pltpu.make_async_copy(stage.at[i], stage.at[i], w_sems.at[i]).wait()

    def run(order, i, **jobs):
        for job in order:
            if job.isdigit():
                project_pair(i, int(job))
            else:
                jobs[job]()

    def norm_body(i, _):
        wait_pair(i)
        got = x_v.at[pl.ds(i * segs, segs)]
        pltpu.make_async_copy(got, got, x_sems.at[i]).wait()
        r0 = pl.multiple_of(i * block, block)

        def prefetch():
            start_pair(i + AHEAD)
            piece(wo_hbm, wo_stage, wo_sems.at[i], i, n_norm).start()

            @pl.when(i + AHEAD < n_norm)
            def _():
                start_x(i + AHEAD)

        norm = []

        def normalise():
            xn = _layernorm(x_v[pl.ds(i * segs, segs)].astype(F32).reshape(block, D))
            xn_v[pl.ds(r0, block), :] = xn
            gin_v[pl.ds(r0, block), :] = xn
            norm.append(xn.astype(BF16))

        def route():
            w_r = wr_v[...].astype(F32)
            w_r = jnp.concatenate(
                [jnp.broadcast_to(w_r[k:k + 1], (8, 128)) for k in range(D // 128)], axis=1)
            score_v[i] = _round(_dot_nt(w_r, norm[0]))

        run(ORDER_A, i, n=normalise, r=route, s=prefetch)

    def pick_body(c, _):
        i = n_norm + c
        wait_pair(i)
        piece(wo_hbm, wo_stage, wo_sems.at[c], c, n_norm).wait()

        def prefetch():
            @pl.when(c < FFN_PIECES)
            def _():
                for k, (src, dst) in enumerate(
                        ((wg_hbm, wg_v), (wu_hbm, wu_v), (wd_hbm, wd_v))):
                    piece(src, dst, misc_sems.at[2 + k], c, FFN_PIECES).start()

            @pl.when(i + AHEAD < n_pair)
            def _():
                start_pair(i + AHEAD)

        def pick():
            score = jnp.concatenate([score_v[j] for j in range(n_norm)], axis=1)
            pos = lax.broadcasted_iota(jnp.int32, (8, S), 1).astype(F32)
            best = jnp.max(jnp.where(score == score, score, -jnp.inf), axis=1, keepdims=True)
            first = jnp.min(jnp.where(score == best, pos, float(S - 1)),
                            axis=1, keepdims=True)
            score = jnp.where(pos == first, jnp.nan, score)
            for j in range(n_norm):
                score_v[j] = score[:, j * block:(j + 1) * block]
            idx = jnp.clip(jnp.max(first).astype(jnp.int32), 0, S - 1)
            picked_s[c] = idx
            xsel_v[pl.ds(c, 1), :] = xn_v[pl.ds(idx, 1), :]
            rsel_v[pl.ds(c, 1), :] = jnp.broadcast_to(best[:1], (1, 128))

        def repack_wo():
            rows = H * DH // TOP_C
            r0 = pl.multiple_of(c * rows, rows)
            p0 = pl.multiple_of(c * (rows // 2), rows // 2)
            wo_v[pl.ds(p0, rows // 2), :] = pltpu.bitcast(wo_stage[pl.ds(r0, rows), :], U32)

        run(ORDER_B, i, p=pick, w=repack_wo, s=prefetch)

    with _scope("dense_a"):
        lax.fori_loop(0, n_norm, norm_body, None)
    with _scope("dense_b"):
        lax.fori_loop(0, TOP_C, pick_body, None)

    pltpu.make_async_copy(wg_hbm, wg_v, misc_sems.at[2]).wait()
    pltpu.make_async_copy(wu_hbm, wu_v, misc_sems.at[3]).wait()
    pltpu.make_async_copy(wd_hbm, wd_v, misc_sems.at[4]).wait()
    x_sel = xsel_v[...]
    act = _round(_silu(_round(_dot_nt(x_sel, wg_v[...]))))
    up = _round(_dot_nt(x_sel, wu_v[...]))
    y = _round(_dot(_round(act * up), wd_v[...]))
    y = _round(y * _round(jax.nn.sigmoid(rsel_v[:, :1])))
    g_in = _round(x_sel + y)
    for c in range(TOP_C):
        gin_v[pl.ds(picked_s[c], 1), :] = g_in[c:c + 1, :]

    n_grp = H // GROUP
    key_pad = -L % 16
    exp_scale = float(DH ** -0.5 * np.log2(np.e))

    def step(s, mem):
        base = pl.multiple_of(s * seg, seg)
        zb = pl.multiple_of(s * HOIST, HOIST)
        h_in = jnp.concatenate([mem, xn_v[pl.ds(base, live), :]], axis=0).astype(BF16)

        row = lax.broadcasted_iota(jnp.int32, (L, L + key_pad), 0)
        col = lax.broadcasted_iota(jnp.int32, (L, L + key_pad), 1)
        visible = ((row < M) | (row >= col)) & (col < L)
        fill = jnp.where(col < L, -1e9 * DH ** 0.5, -jnp.inf).astype(F32)

        qkv, prob, ctx, acc = {}, {}, {}, []

        def keys(t):
            return jnp.concatenate([t, jnp.zeros((key_pad, DH), F32)], axis=0).astype(BF16)

        def project(g):
            ids = [m * H + h for h in range(g * GROUP, (g + 1) * GROUP) for m in range(3)]
            if g == 0 and K_MAJOR:
                y = functools.reduce(lambda a, b: a + b, [
                    _dot(h_in[:, k * 128:(k + 1) * 128], jnp.concatenate(
                        [pltpu.bitcast(wqkv[i, k * 64:(k + 1) * 64, :], BF16) for i in ids],
                        axis=1))
                    for k in range(D // 128)])
            else:
                y = _dot(h_in, jnp.concatenate(
                    [pltpu.bitcast(wqkv[i], BF16) for i in ids], axis=1))
            for j, i in enumerate(ids):
                qkv[i] = jnp.concatenate(
                    [y[:, j * DH:(j + 1) * DH], hz[i, pl.ds(zb, HOIST), :]], axis=0)

        def scores(g):
            for h in range(g * GROUP, (g + 1) * GROUP):
                sc = _dot_nt(_round(qkv[h]), keys(qkv[H + h]))
                sc = jnp.where(visible, sc, fill)
                e = jnp.exp2((sc - jnp.max(sc, axis=1, keepdims=True)) * exp_scale)
                prob[h] = _round(e / jnp.sum(e, axis=1, keepdims=True))

        def values(g):
            for h in range(g * GROUP, (g + 1) * GROUP):
                ctx[h] = _round(_dot(prob[h], keys(qkv[2 * H + h])))

        def out_proj(lo, hi):
            o = jnp.concatenate([ctx[h] for h in range(lo * GROUP, hi * GROUP)], axis=1)
            rows = GROUP * DH // 2
            if hi == n_grp and N_MAJOR:
                acc.append(jnp.concatenate([
                    _dot(o, pltpu.bitcast(
                        wo_v[lo * rows:hi * rows, n * 128:(n + 1) * 128], BF16))
                    for n in range(D // 128)], axis=1))
            else:
                acc.append(_dot(o, pltpu.bitcast(wo_v[lo * rows:hi * rows, :], BF16)))

        for t in range(n_grp):
            project(t)
            if t >= LAG_QK:
                scores(t - LAG_QK)
            if t >= LAG_QK + LAG_PV:
                values(t - LAG_QK - LAG_PV)
        for op in TAIL.split("-"):
            if op[0] == "S":
                scores(int(op[1:]))
            elif op[0] == "V":
                values(int(op[1:]))
            else:
                out_proj(*map(int, op[1:].split(":")))

        o = functools.reduce(lambda a, b: a + b, acc)
        gate = _silu(gin_v[pl.ds(base, seg), :])
        out_v[s] = (x_v[s].astype(F32) + o[M:] * gate).astype(BF16)
        pltpu.make_async_copy(out_v.at[s], out_hbm.at[s], out_sem).start()
        return _round(o[:M])

    mem0_cp.wait()
    with _scope("steps"):
        lax.fori_loop(0, n_seg, step, mem0_v[...].astype(F32), unroll=UNROLL)
    pltpu.make_async_copy(out_v, out_hbm, out_sem).wait()


@functools.partial(jax.jit, static_argnames=("A_seg_len",))
def pallas_recurrent_scan__memory_aug_recurrent_mem_tr__moe_arch_mod__prompt_kernel(
    A_x: jax.Array,
    A_mem0: jax.Array,
    A_Wq: jax.Array,
    A_Wk: jax.Array,
    A_Wv: jax.Array,
    A_Wo: jax.Array,
    A_seg_len: int,
    B_x: jax.Array,
    B_w_r: jax.Array,
    B_w_gate: jax.Array,
    B_w_up: jax.Array,
    B_w_down: jax.Array,
):
    del B_x
    B, S, D = A_x.shape
    M = A_mem0.shape[1]
    _, H, DH = A_Wq.shape
    F = B_w_gate.shape[1]
    seg = int(A_seg_len)
    n_seg = S // seg
    n_norm = H // 2 - TOP_C
    assert B == 1 and M == 8 and DH == 128 and seg % 16 == 0 and n_seg * seg == S

    hbm = pl.BlockSpec(memory_space=pltpu.HBM)
    out = pl.pallas_call(
        _kernel,
        out_shape=jax.ShapeDtypeStruct((n_seg, seg, D), A_x.dtype),
        in_specs=[hbm] * 10,
        out_specs=hbm,
        scratch_shapes=[
            pltpu.VMEM((n_seg, seg, D), BF16),
            pltpu.VMEM((n_seg, HOIST, D), BF16),
            pltpu.VMEM((M, D), BF16),
            pltpu.VMEM((D // 128, 128), BF16),
            pltpu.VMEM((S, D), F32),
            pltpu.VMEM((S, D), F32),
            pltpu.VMEM((n_seg * HOIST, D), BF16),
            pltpu.VMEM((H // 2, 3, D, DH), U32),
            pltpu.VMEM((3 * H, D // 2, DH), U32),
            pltpu.VMEM((H * DH, D), BF16),
            pltpu.VMEM((H * DH // 2, D), U32),
            pltpu.VMEM((3 * H, n_seg * HOIST, DH), F32),
            pltpu.VMEM((F, D), BF16),
            pltpu.VMEM((F, D), BF16),
            pltpu.VMEM((F, D), BF16),
            pltpu.VMEM((n_seg, seg, D), BF16),
            pltpu.VMEM((n_norm, 8, S // n_norm), F32),
            pltpu.VMEM((TOP_C, D), F32),
            pltpu.VMEM((TOP_C, 128), F32),
            pltpu.SMEM((TOP_C,), jnp.int32),
            pltpu.SemaphoreType.DMA((n_norm,)),
            pltpu.SemaphoreType.DMA((H // 2,)),
            pltpu.SemaphoreType.DMA((n_norm,)),
            pltpu.SemaphoreType.DMA((7,)),
            pltpu.SemaphoreType.DMA(()),
        ],
        compiler_params=pltpu.CompilerParams(vmem_limit_bytes=112 * 1024 * 1024),
    )(A_x.reshape(n_seg, seg, D), A_mem0.reshape(M, D), A_Wq, A_Wk, A_Wv,
      A_Wo.reshape(H * DH, D), B_w_r.reshape(D // 128, 128), B_w_gate.T, B_w_up.T, B_w_down)
    return out.reshape(B, S, D)
```

```python
import functools

import jax
import jax.numpy as jnp
import numpy as np
from jax import lax
from jax.experimental import pallas as pl
from jax.experimental.pallas import tpu as pltpu

F32 = jnp.float32
BF16 = jnp.bfloat16
U32 = jnp.uint32

TOP_C = 8
HOIST = 8
NO_CHECKS = 0
PICKS = 2
SINGLES = 8
AHEAD = 4
GROUP = 4
LAG_QK = 1
LAG_PV = 1
TAIL = "S7-O0:2-O2:4-V6-V7-O4:6-O6:8"
UNROLL = 8
ORDER_A = "n012rs"
ORDER_A2 = "n012345rs"
ORDER_B = "0p1w2345s"
K_MAJOR = 1
N_MAJOR = 1
PROFILE = 0


def _scope(name):
    import contextlib
    return jax.named_scope(name) if PROFILE else contextlib.nullcontext()


def _dot(a, b):
    return lax.dot_general(a, b, (((1,), (0,)), ((), ())), preferred_element_type=F32)


def _dot_nt(a, b):
    return lax.dot_general(a, b, (((1,), (1,)), ((), ())), preferred_element_type=F32)


def _round(x):
    return x.astype(BF16).astype(F32)


def _silu(x):
    h = 0.5 * x
    return h + h * jnp.tanh(h)


def _layernorm(x):
    inv_n = 1.0 / x.shape[-1]
    mean = jnp.sum(x, axis=-1, keepdims=True) * inv_n
    cen = x - mean
    var = jnp.sum(cen * cen, axis=-1, keepdims=True) * inv_n
    eps = float(np.asarray(1e-5, dtype=BF16))
    sd = _round(jnp.sqrt(_round(_round(var) + eps)))
    return _round(_round(x - _round(mean)) * (1.0 / sd))


def _kernel(x_hbm, mem0_hbm, wq_hbm, wk_hbm, wv_hbm, wo_hbm, wr_hbm, wg_hbm, wu_hbm, wd_hbm,
            out_hbm,
            x_v, xh_raw, mem0_v, wr_v, xn_v, gin_v, xh_v, stage, wqkv, wo_stage, wo_v, hz,
            wg_v, wu_v, wd_v, out_v, score_v, xsel_v, rsel_v, picked_s,
            x_sems, w_sems, wo_sems, misc_sems, out_sem):
    n_seg, seg, D = x_v.shape
    S = n_seg * seg
    M = mem0_v.shape[0]
    H, DH = wq_hbm.shape[1], wq_hbm.shape[2]
    L = M + seg
    live = seg - HOIST
    n_pair = H // 2
    n_norm = n_pair - TOP_C
    segs = n_seg // n_norm
    block = segs * seg

    words = [w.bitcast(U32) for w in (wq_hbm, wk_hbm, wv_hbm)]

    def start_pair(i):
        for m in range(3):
            pltpu.make_async_copy(words[m].at[:, i, :], stage.at[i, m], w_sems.at[i]).start()

    def start_x(i):
        at = pl.ds(i * segs, segs)
        pltpu.make_async_copy(x_hbm.at[at], x_v.at[at], x_sems.at[i]).start()

    def piece(src, dst, sem, i, n):
        rows = dst.shape[0] // n
        at = pl.ds(pl.multiple_of(i * rows, 8), rows)
        return pltpu.make_async_copy(src.at[at], dst.at[at], sem)

    xh_cp = pltpu.make_async_copy(x_hbm.at[:, pl.ds(live, HOIST), :], xh_raw, misc_sems.at[0])
    mem0_cp = pltpu.make_async_copy(mem0_hbm, mem0_v, misc_sems.at[5])
    wr_cp = pltpu.make_async_copy(wr_hbm, wr_v, misc_sems.at[6])
    ffn_cps = [pltpu.make_async_copy(src, dst, misc_sems.at[2 + j]) for j, (src, dst)
               in enumerate(((wg_hbm, wg_v), (wu_hbm, wu_v), (wd_hbm, wd_v)))]
    xh_cp.start()
    start_pair(0)
    start_x(0)
    wr_cp.start()

    with _scope("xh_wait"):
        xh_cp.wait()
    start_pair(1)
    start_x(1)
    mem0_cp.start()

    def xh_body(i, _):
        s0 = pl.multiple_of(i * 16, 16)
        rows = xh_raw[pl.ds(s0, 16)].astype(F32).reshape(16 * HOIST, D)
        r0 = pl.multiple_of(i * (16 * HOIST), 16 * HOIST)
        xh_v[pl.ds(r0, 16 * HOIST), :] = _layernorm(rows).astype(BF16)

    with _scope("xh_ln"):
        lax.fori_loop(0, n_seg // 16, xh_body, None)
    wr_cp.wait()
    for i in range(2, AHEAD):
        start_pair(i)
        start_x(i)

    def project_pair(i, m):
        a = stage[i, m, pl.ds(0, D // 2, stride=2), :]
        b = stage[i, m, pl.ds(1, D // 2, stride=2), :]
        even = (a & jnp.uint32(0xFFFF)) | (b << 16)
        odd = (a >> 16) | (b & jnp.uint32(0xFFFF0000))
        head = m * H + 2 * i
        wqkv[head] = even
        wqkv[head + 1] = odd
        w = jnp.concatenate([pltpu.bitcast(even, BF16), pltpu.bitcast(odd, BF16)], axis=1)
        y = _dot(xh_v[...], w)
        hz[head] = y[:, :DH]
        hz[head + 1] = y[:, DH:]

    def wait_pair(i):
        pltpu.make_async_copy(stage.at[i], stage.at[i], w_sems.at[i]).wait()

    def run(order, i, **jobs):
        for job in order:
            if job.isdigit():
                project_pair(i + int(job) // 3, int(job) % 3)
            else:
                jobs[job]()

    def norm_body(t, _, *, first, n):
        i = first + t * n
        for k in range(n):
            wait_pair(i + k)
            got = x_v.at[pl.ds((i + k) * segs, segs)]
            pltpu.make_async_copy(got, got, x_sems.at[i + k]).wait()
        r0 = pl.multiple_of(i * block, block)
        norm = []

        def normalise():
            x = x_v[pl.ds(i * segs, n * segs)].astype(F32).reshape(n * block, D)
            xn = _layernorm(x)
            xn_v[pl.ds(r0, n * block), :] = xn
            gin_v[pl.ds(r0, n * block), :] = xn
            norm.append(xn.astype(BF16))

        def route():
            w_r = wr_v[...].astype(F32)
            w_r = jnp.concatenate(
                [jnp.broadcast_to(w_r[k:k + 1], (8, 128)) for k in range(D // 128)], axis=1)
            score = _round(_dot_nt(w_r, norm[0]))
            for k in range(n):
                score_v[i + k] = score[:, k * block:(k + 1) * block]

        def prefetch():
            for k in range(n):
                start_pair(i + k + AHEAD)
                piece(wo_hbm, wo_stage, wo_sems.at[i + k], i + k, n_norm).start()

            @pl.when(i + AHEAD < n_norm)
            def _():
                for k in range(n):
                    start_x(i + k + AHEAD)

        run(ORDER_A if n == 1 else ORDER_A2, i, n=normalise, r=route, s=prefetch)

    def pick_body(t, _, *, n):
        c = t * n
        i = n_norm + c
        for k in range(n):
            wait_pair(i + k)
            piece(wo_hbm, wo_stage, wo_sems.at[c + k], c + k, n_norm).wait()

        def prefetch():
            for j, cp in enumerate(ffn_cps):
                pl.when(t == j)(cp.start)

        def pick():
            score = jnp.concatenate([score_v[j] for j in range(n_norm)], axis=1)
            pos = lax.broadcasted_iota(jnp.int32, (8, S), 1).astype(F32)
            for k in range(n):
                best = jnp.max(jnp.where(score == score, score, -jnp.inf),
                               axis=1, keepdims=True)
                first = jnp.min(jnp.where(score == best, pos, float(S - 1)),
                                axis=1, keepdims=True)
                score = jnp.where(pos == first, jnp.nan, score)
                idx = jnp.clip(jnp.max(first).astype(jnp.int32), 0, S - 1)
                picked_s[c + k] = idx
                xsel_v[pl.ds(c + k, 1), :] = xn_v[pl.ds(idx, 1), :]
                rsel_v[pl.ds(c + k, 1), :] = jnp.broadcast_to(best[:1], (1, 128))
            for j in range(n_norm):
                score_v[j] = score[:, j * block:(j + 1) * block]

        def repack_wo():
            rows = H * DH // n_norm
            r0 = pl.multiple_of(c * rows, n * rows)
            p0 = pl.multiple_of(c * (rows // 2), n * rows // 2)
            wo_v[pl.ds(p0, n * rows // 2), :] = pltpu.bitcast(
                wo_stage[pl.ds(r0, n * rows), :], U32)

        run(ORDER_B, i, p=pick, w=repack_wo, s=prefetch)

    with _scope("dense_a"):
        lax.fori_loop(0, SINGLES, functools.partial(norm_body, first=0, n=1), None)
    if SINGLES < n_norm:
        lax.fori_loop(0, (n_norm - SINGLES) // 2,
                      functools.partial(norm_body, first=SINGLES, n=2), None)
    for i in range(n_norm + AHEAD, n_pair):
        start_pair(i)
    with _scope("dense_b"):
        lax.fori_loop(0, TOP_C // PICKS, functools.partial(pick_body, n=PICKS), None)

    for cp in ffn_cps:
        cp.wait()
    x_sel = xsel_v[...]
    act = _round(_silu(_round(_dot_nt(x_sel, wg_v[...]))))
    up = _round(_dot_nt(x_sel, wu_v[...]))
    y = _round(_dot(_round(act * up), wd_v[...]))
    y = _round(y * _round(jax.nn.sigmoid(rsel_v[:, :1])))
    g_in = _round(x_sel + y)
    for c in range(TOP_C):
        gin_v[pl.ds(picked_s[c], 1), :] = g_in[c:c + 1, :]

    n_grp = H // GROUP
    key_pad = -L % 16
    exp_scale = float(DH ** -0.5 * np.log2(np.e))

    def step(s, mem):
        base = pl.multiple_of(s * seg, seg)
        zb = pl.multiple_of(s * HOIST, HOIST)
        h_in = jnp.concatenate([mem, xn_v[pl.ds(base, live), :]], axis=0).astype(BF16)

        row = lax.broadcasted_iota(jnp.int32, (L, L + key_pad), 0)
        col = lax.broadcasted_iota(jnp.int32, (L, L + key_pad), 1)
        visible = ((row < M) | (row >= col)) & (col < L)
        fill = jnp.where(col < L, -1e9 * DH ** 0.5, -jnp.inf).astype(F32)

        qkv, prob, ctx, acc = {}, {}, {}, []

        def keys(t):
            return jnp.concatenate([t, jnp.zeros((key_pad, DH), F32)], axis=0).astype(BF16)

        def project(g):
            ids = [m * H + h for h in range(g * GROUP, (g + 1) * GROUP) for m in range(3)]
            if g == 0 and K_MAJOR:
                y = functools.reduce(lambda a, b: a + b, [
                    _dot(h_in[:, k * 128:(k + 1) * 128], jnp.concatenate(
                        [pltpu.bitcast(wqkv[i, k * 64:(k + 1) * 64, :], BF16) for i in ids],
                        axis=1))
                    for k in range(D // 128)])
            else:
                y = _dot(h_in, jnp.concatenate(
                    [pltpu.bitcast(wqkv[i], BF16) for i in ids], axis=1))
            for j, i in enumerate(ids):
                qkv[i] = jnp.concatenate(
                    [y[:, j * DH:(j + 1) * DH], hz[i, pl.ds(zb, HOIST), :]], axis=0)

        def scores(g):
            for h in range(g * GROUP, (g + 1) * GROUP):
                sc = _dot_nt(_round(qkv[h]), keys(qkv[H + h]))
                sc = jnp.where(visible, sc, fill)
                e = jnp.exp2((sc - jnp.max(sc, axis=1, keepdims=True)) * exp_scale)
                prob[h] = _round(e / jnp.sum(e, axis=1, keepdims=True))

        def values(g):
            for h in range(g * GROUP, (g + 1) * GROUP):
                ctx[h] = _round(_dot(prob[h], keys(qkv[2 * H + h])))

        def out_proj(lo, hi):
            o = jnp.concatenate([ctx[h] for h in range(lo * GROUP, hi * GROUP)], axis=1)
            rows = GROUP * DH // 2
            if hi == n_grp and N_MAJOR:
                acc.append(jnp.concatenate([
                    _dot(o, pltpu.bitcast(
                        wo_v[lo * rows:hi * rows, n * 128:(n + 1) * 128], BF16))
                    for n in range(D // 128)], axis=1))
            else:
                acc.append(_dot(o, pltpu.bitcast(wo_v[lo * rows:hi * rows, :], BF16)))

        for t in range(n_grp):
            project(t)
            if t >= LAG_QK:
                scores(t - LAG_QK)
            if t >= LAG_QK + LAG_PV:
                values(t - LAG_QK - LAG_PV)
        for op in TAIL.split("-"):
            if op[0] == "S":
                scores(int(op[1:]))
            elif op[0] == "V":
                values(int(op[1:]))
            else:
                out_proj(*map(int, op[1:].split(":")))

        o = functools.reduce(lambda a, b: a + b, acc)
        gate = _silu(gin_v[pl.ds(base, seg), :])
        out_v[s] = (x_v[s].astype(F32) + o[M:] * gate).astype(BF16)
        pltpu.make_async_copy(out_v.at[s], out_hbm.at[s], out_sem).start()
        return _round(o[:M])

    mem0_cp.wait()
    with _scope("steps"):
        lax.fori_loop(0, n_seg, step, mem0_v[...].astype(F32), unroll=UNROLL)
    pltpu.make_async_copy(out_v, out_hbm, out_sem).wait()


@functools.partial(jax.jit, static_argnames=("A_seg_len",))
def pallas_recurrent_scan__memory_aug_recurrent_mem_tr__moe_arch_mod__prompt_kernel(
    A_x: jax.Array,
    A_mem0: jax.Array,
    A_Wq: jax.Array,
    A_Wk: jax.Array,
    A_Wv: jax.Array,
    A_Wo: jax.Array,
    A_seg_len: int,
    B_x: jax.Array,
    B_w_r: jax.Array,
    B_w_gate: jax.Array,
    B_w_up: jax.Array,
    B_w_down: jax.Array,
):
    del B_x
    B, S, D = A_x.shape
    M = A_mem0.shape[1]
    _, H, DH = A_Wq.shape
    F = B_w_gate.shape[1]
    seg = int(A_seg_len)
    n_seg = S // seg
    n_norm = H // 2 - TOP_C
    assert B == 1 and M == 8 and DH == 128 and seg % 16 == 0 and n_seg * seg == S

    hbm = pl.BlockSpec(memory_space=pltpu.HBM)
    out = pl.pallas_call(
        _kernel,
        out_shape=jax.ShapeDtypeStruct((n_seg, seg, D), A_x.dtype),
        in_specs=[hbm] * 10,
        out_specs=hbm,
        scratch_shapes=[
            pltpu.VMEM((n_seg, seg, D), BF16),
            pltpu.VMEM((n_seg, HOIST, D), BF16),
            pltpu.VMEM((M, D), BF16),
            pltpu.VMEM((D // 128, 128), BF16),
            pltpu.VMEM((S, D), F32),
            pltpu.VMEM((S, D), F32),
            pltpu.VMEM((n_seg * HOIST, D), BF16),
            pltpu.VMEM((H // 2, 3, D, DH), U32),
            pltpu.VMEM((3 * H, D // 2, DH), U32),
            pltpu.VMEM((H * DH, D), BF16),
            pltpu.VMEM((H * DH // 2, D), U32),
            pltpu.VMEM((3 * H, n_seg * HOIST, DH), F32),
            pltpu.VMEM((F, D), BF16),
            pltpu.VMEM((F, D), BF16),
            pltpu.VMEM((F, D), BF16),
            pltpu.VMEM((n_seg, seg, D), BF16),
            pltpu.VMEM((n_norm, 8, S // n_norm), F32),
            pltpu.VMEM((TOP_C, D), F32),
            pltpu.VMEM((TOP_C, 128), F32),
            pltpu.SMEM((TOP_C,), jnp.int32),
            pltpu.SemaphoreType.DMA((n_norm,)),
            pltpu.SemaphoreType.DMA((H // 2,)),
            pltpu.SemaphoreType.DMA((n_norm,)),
            pltpu.SemaphoreType.DMA((7,)),
            pltpu.SemaphoreType.DMA(()),
        ],
        compiler_params=pltpu.CompilerParams(vmem_limit_bytes=112 * 1024 * 1024,
                                             disable_bounds_checks=bool(NO_CHECKS)),
    )(A_x.reshape(n_seg, seg, D), A_mem0.reshape(M, D), A_Wq, A_Wk, A_Wv,
      A_Wo.reshape(H * DH, D), B_w_r.reshape(D // 128, 128), B_w_gate.T, B_w_up.T, B_w_down)
    return out.reshape(B, S, D)
```

```python
import functools

import jax
import jax.numpy as jnp
import numpy as np
from jax import lax
from jax.experimental import pallas as pl
from jax.experimental.pallas import tpu as pltpu

F32 = jnp.float32
BF16 = jnp.bfloat16
U32 = jnp.uint32

TOP_C = 8
HOIST = 8
AHEAD = 4
PICKS = 2
GROUP = 4
UNROLL = 8


def _dot(a, b):
    return lax.dot_general(a, b, (((1,), (0,)), ((), ())), preferred_element_type=F32)


def _dot_nt(a, b):
    return lax.dot_general(a, b, (((1,), (1,)), ((), ())), preferred_element_type=F32)


def _total(terms):
    return functools.reduce(lambda a, b: a + b, terms)


def _round(x):
    return x.astype(BF16).astype(F32)


def _silu(x):
    h = 0.5 * x
    return h + h * jnp.tanh(h)


def _layernorm(x):
    inv_n = 1.0 / x.shape[-1]
    mean = jnp.sum(x, axis=-1, keepdims=True) * inv_n
    cen = x - mean
    var = jnp.sum(cen * cen, axis=-1, keepdims=True) * inv_n
    eps = float(np.asarray(1e-5, dtype=BF16))
    sd = _round(jnp.sqrt(_round(_round(var) + eps)))
    return _round(_round(x - _round(mean)) * (1.0 / sd))


def _kernel(x_hbm, mem0_hbm, wq_hbm, wk_hbm, wv_hbm, wo_hbm, wr_hbm, wg_hbm, wu_hbm, wd_hbm,
            out_hbm,
            x_v, xh_raw, mem0_v, wr_v, xn_v, gin_v, xh_v, stage, wqkv, wo_stage, wo_v, hz,
            wg_v, wu_v, wd_v, out_v, score_v, xsel_v, rsel_v, picked_s,
            x_sems, w_sems, wo_sems, misc_sems, out_sem):
    n_seg, seg, D = x_v.shape
    S = n_seg * seg
    M = mem0_v.shape[0]
    H, DH = wq_hbm.shape[1], wq_hbm.shape[2]
    L = M + seg
    live = seg - HOIST
    n_pair = H // 2
    n_norm = n_pair - TOP_C
    segs = n_seg // n_norm
    block = segs * seg

    words = [w.bitcast(U32) for w in (wq_hbm, wk_hbm, wv_hbm)]

    def start_pair(i):
        for m in range(3):
            pltpu.make_async_copy(words[m].at[:, i, :], stage.at[i, m], w_sems.at[i]).start()

    def wait_pair(i):
        pltpu.make_async_copy(stage.at[i], stage.at[i], w_sems.at[i]).wait()

    def x_copy(i):
        at = pl.ds(i * segs, segs)
        return pltpu.make_async_copy(x_hbm.at[at], x_v.at[at], x_sems.at[i])

    def wo_copy(i):
        rows = H * DH // n_norm
        at = pl.ds(pl.multiple_of(i * rows, rows), rows)
        return pltpu.make_async_copy(wo_hbm.at[at], wo_stage.at[at], wo_sems.at[i])

    xh_cp = pltpu.make_async_copy(x_hbm.at[:, pl.ds(live, HOIST), :], xh_raw, misc_sems.at[0])
    mem0_cp = pltpu.make_async_copy(mem0_hbm, mem0_v, misc_sems.at[1])
    wr_cp = pltpu.make_async_copy(wr_hbm, wr_v, misc_sems.at[2])
    ffn_cps = [pltpu.make_async_copy(src, dst, misc_sems.at[3 + j]) for j, (src, dst)
               in enumerate(((wg_hbm, wg_v), (wu_hbm, wu_v), (wd_hbm, wd_v)))]
    xh_cp.start()
    start_pair(0)
    x_copy(0).start()
    wr_cp.start()

    xh_cp.wait()
    start_pair(1)
    x_copy(1).start()
    mem0_cp.start()

    def xh_body(i, _):
        s0 = pl.multiple_of(i * 16, 16)
        rows = xh_raw[pl.ds(s0, 16)].astype(F32).reshape(16 * HOIST, D)
        r0 = pl.multiple_of(i * (16 * HOIST), 16 * HOIST)
        xh_v[pl.ds(r0, 16 * HOIST), :] = _layernorm(rows).astype(BF16)

    lax.fori_loop(0, n_seg // 16, xh_body, None)
    wr_cp.wait()
    for i in range(2, AHEAD):
        start_pair(i)
        x_copy(i).start()

    def project_pair(i, m):
        a = stage[i, m, pl.ds(0, D // 2, stride=2), :]
        b = stage[i, m, pl.ds(1, D // 2, stride=2), :]
        even = (a & jnp.uint32(0xFFFF)) | (b << 16)
        odd = (a >> 16) | (b & jnp.uint32(0xFFFF0000))
        head = m * H + 2 * i
        wqkv[head] = even
        wqkv[head + 1] = odd
        w = jnp.concatenate([pltpu.bitcast(even, BF16), pltpu.bitcast(odd, BF16)], axis=1)
        y = _dot(xh_v[...], w)
        hz[head] = y[:, :DH]
        hz[head + 1] = y[:, DH:]

    def norm_body(i, _):
        wait_pair(i)
        x_copy(i).wait()

        xn = _layernorm(x_v[pl.ds(i * segs, segs)].astype(F32).reshape(block, D))
        r0 = pl.multiple_of(i * block, block)
        xn_v[pl.ds(r0, block), :] = xn
        gin_v[pl.ds(r0, block), :] = xn
        xn = xn.astype(BF16)

        for m in range(3):
            project_pair(i, m)

        w_r = wr_v[...].astype(F32)
        w_r = jnp.concatenate(
            [jnp.broadcast_to(w_r[k:k + 1], (8, 128)) for k in range(D // 128)], axis=1)
        score_v[i] = _round(_dot_nt(w_r, xn))

        start_pair(i + AHEAD)
        wo_copy(i).start()

        @pl.when(i + AHEAD < n_norm)
        def _():
            x_copy(i + AHEAD).start()

    def pick_body(t, _):
        c = t * PICKS
        i = n_norm + c
        for k in range(PICKS):
            wait_pair(i + k)
            wo_copy(c + k).wait()

        project_pair(i, 0)

        score = jnp.concatenate([score_v[j] for j in range(n_norm)], axis=1)
        pos = lax.broadcasted_iota(jnp.int32, (8, S), 1).astype(F32)
        for k in range(PICKS):
            best = jnp.max(jnp.where(score == score, score, -jnp.inf), axis=1, keepdims=True)
            first = jnp.min(jnp.where(score == best, pos, float(S - 1)),
                            axis=1, keepdims=True)
            score = jnp.where(pos == first, jnp.nan, score)
            idx = jnp.clip(jnp.max(first).astype(jnp.int32), 0, S - 1)
            picked_s[c + k] = idx
            xsel_v[pl.ds(c + k, 1), :] = xn_v[pl.ds(idx, 1), :]
            rsel_v[pl.ds(c + k, 1), :] = jnp.broadcast_to(best[:1], (1, 128))
        for j in range(n_norm):
            score_v[j] = score[:, j * block:(j + 1) * block]

        project_pair(i, 1)

        rows = PICKS * H * DH // n_norm
        r0 = pl.multiple_of(t * rows, rows)
        p0 = pl.multiple_of(t * (rows // 2), rows // 2)
        wo_v[pl.ds(p0, rows // 2), :] = pltpu.bitcast(wo_stage[pl.ds(r0, rows), :], U32)

        for j in range(2, 3 * PICKS):
            project_pair(i + j // 3, j % 3)

        for j, cp in enumerate(ffn_cps):
            pl.when(t == j)(cp.start)

    lax.fori_loop(0, n_norm, norm_body, None)
    for i in range(n_norm + AHEAD, n_pair):
        start_pair(i)
    lax.fori_loop(0, TOP_C // PICKS, pick_body, None)

    for cp in ffn_cps:
        cp.wait()
    x_sel = xsel_v[...]
    act = _round(_silu(_round(_dot_nt(x_sel, wg_v[...]))))
    up = _round(_dot_nt(x_sel, wu_v[...]))
    y = _round(_dot(_round(act * up), wd_v[...]))
    y = _round(y * _round(jax.nn.sigmoid(rsel_v[:, :1])))
    g_in = _round(x_sel + y)
    for c in range(TOP_C):
        gin_v[pl.ds(jnp.clip(picked_s[c], 0, S - 1), 1), :] = g_in[c:c + 1, :]

    n_grp = H // GROUP
    key_pad = -L % 16
    exp_scale = float(DH ** -0.5 * np.log2(np.e))

    def step(s, mem):
        base = pl.multiple_of(s * seg, seg)
        zb = pl.multiple_of(s * HOIST, HOIST)
        h_in = jnp.concatenate([mem, xn_v[pl.ds(base, live), :]], axis=0).astype(BF16)

        row = lax.broadcasted_iota(jnp.int32, (L, L + key_pad), 0)
        col = lax.broadcasted_iota(jnp.int32, (L, L + key_pad), 1)
        visible = ((row < M) | (row >= col)) & (col < L)
        fill = jnp.where(col < L, -1e9 * DH ** 0.5, -jnp.inf).astype(F32)

        qkv, prob, ctx, parts = {}, {}, {}, []

        def keys(t):
            return jnp.concatenate([t, jnp.zeros((key_pad, DH), F32)], axis=0).astype(BF16)

        def project(g):
            ids = [m * H + h for m in (1, 0, 2) for h in range(g * GROUP, (g + 1) * GROUP)]
            if g == 0:
                y = _total([
                    _dot(h_in[:, k * 128:(k + 1) * 128], jnp.concatenate(
                        [pltpu.bitcast(wqkv[i, k * 64:(k + 1) * 64, :], BF16) for i in ids],
                        axis=1))
                    for k in range(D // 128)])
            else:
                y = _dot(h_in, jnp.concatenate(
                    [pltpu.bitcast(wqkv[i], BF16) for i in ids], axis=1))
            for j, i in enumerate(ids):
                qkv[i] = jnp.concatenate(
                    [y[:, j * DH:(j + 1) * DH], hz[i, pl.ds(zb, HOIST), :]], axis=0)

        def scores(g):
            for h in range(g * GROUP, (g + 1) * GROUP):
                sc = _dot_nt(_round(qkv[h]), keys(qkv[H + h]))
                sc = jnp.where(visible, sc, fill)
                e = jnp.exp2((sc - jnp.max(sc, axis=1, keepdims=True)) * exp_scale)
                prob[h] = _round(e / jnp.sum(e, axis=1, keepdims=True))

        def values(g):
            for h in range(g * GROUP, (g + 1) * GROUP):
                ctx[h] = _round(_dot(prob[h], keys(qkv[2 * H + h])))

        def out_proj(lo, hi):
            o = jnp.concatenate([ctx[h] for h in range(lo * GROUP, hi * GROUP)], axis=1)
            rows = GROUP * DH // 2
            parts.append(_dot(o, pltpu.bitcast(wo_v[lo * rows:hi * rows, :], BF16)))

        for g in range(n_grp):
            project(g)
            if g >= 1:
                scores(g - 1)
            if g >= 2:
                values(g - 2)
        scores(n_grp - 1)
        out_proj(0, n_grp // 4)
        out_proj(n_grp // 4, n_grp // 2)
        values(n_grp - 2)
        values(n_grp - 1)
        out_proj(n_grp // 2, n_grp)

        o = _total(parts)
        gate = _silu(gin_v[pl.ds(base, seg), :])
        out_v[s] = (x_v[s].astype(F32) + o[M:] * gate).astype(BF16)
        pltpu.make_async_copy(out_v.at[s], out_hbm.at[s], out_sem).start()
        return _round(o[:M])

    mem0_cp.wait()
    lax.fori_loop(0, n_seg, step, mem0_v[...].astype(F32), unroll=UNROLL)
    pltpu.make_async_copy(out_v, out_hbm, out_sem).wait()


@functools.partial(jax.jit, static_argnames=("A_seg_len",))
def pallas_recurrent_scan__memory_aug_recurrent_mem_tr__moe_arch_mod__prompt_kernel(
    A_x: jax.Array,
    A_mem0: jax.Array,
    A_Wq: jax.Array,
    A_Wk: jax.Array,
    A_Wv: jax.Array,
    A_Wo: jax.Array,
    A_seg_len: int,
    B_x: jax.Array,
    B_w_r: jax.Array,
    B_w_gate: jax.Array,
    B_w_up: jax.Array,
    B_w_down: jax.Array,
):
    del B_x
    B, S, D = A_x.shape
    M = A_mem0.shape[1]
    _, H, DH = A_Wq.shape
    F = B_w_gate.shape[1]
    seg = int(A_seg_len)
    n_seg = S // seg
    n_norm = H // 2 - TOP_C
    assert B == 1 and M == 8 and DH == 128 and D % 128 == 0 and H % (4 * GROUP) == 0
    assert seg % 16 == 0 and n_seg * seg == S and n_seg % 16 == 0
    assert n_norm == TOP_C and n_seg % n_norm == 0 and TOP_C // PICKS > 3

    hbm = pl.BlockSpec(memory_space=pltpu.HBM)
    out = pl.pallas_call(
        _kernel,
        out_shape=jax.ShapeDtypeStruct((n_seg, seg, D), A_x.dtype),
        in_specs=[hbm] * 10,
        out_specs=hbm,
        scratch_shapes=[
            pltpu.VMEM((n_seg, seg, D), BF16),
            pltpu.VMEM((n_seg, HOIST, D), BF16),
            pltpu.VMEM((M, D), BF16),
            pltpu.VMEM((D // 128, 128), BF16),
            pltpu.VMEM((S, D), F32),
            pltpu.VMEM((S, D), F32),
            pltpu.VMEM((n_seg * HOIST, D), BF16),
            pltpu.VMEM((H // 2, 3, D, DH), U32),
            pltpu.VMEM((3 * H, D // 2, DH), U32),
            pltpu.VMEM((H * DH, D), BF16),
            pltpu.VMEM((H * DH // 2, D), U32),
            pltpu.VMEM((3 * H, n_seg * HOIST, DH), F32),
            pltpu.VMEM((F, D), BF16),
            pltpu.VMEM((F, D), BF16),
            pltpu.VMEM((F, D), BF16),
            pltpu.VMEM((n_seg, seg, D), BF16),
            pltpu.VMEM((n_norm, 8, S // n_norm), F32),
            pltpu.VMEM((TOP_C, D), F32),
            pltpu.VMEM((TOP_C, 128), F32),
            pltpu.SMEM((TOP_C,), jnp.int32),
            pltpu.SemaphoreType.DMA((n_norm,)),
            pltpu.SemaphoreType.DMA((H // 2,)),
            pltpu.SemaphoreType.DMA((n_norm,)),
            pltpu.SemaphoreType.DMA((6,)),
            pltpu.SemaphoreType.DMA(()),
        ],
        compiler_params=pltpu.CompilerParams(vmem_limit_bytes=112 * 1024 * 1024),
    )(A_x.reshape(n_seg, seg, D), A_mem0.reshape(M, D), A_Wq, A_Wk, A_Wv,
      A_Wo.reshape(H * DH, D), B_w_r.reshape(D // 128, 128), B_w_gate.T, B_w_up.T, B_w_down)
    return out.reshape(B, S, D)
```
